```python
import os as _os
_os.environ.setdefault("JAX_PLATFORMS", "cpu")
import jax
import jax.numpy as jnp

def _softmax(x, axis=-1):
    return jax.nn.softmax(x, axis=axis)
def _gelu(x):
    return jax.nn.gelu(x, approximate=True)
def _silu(x):
    return jax.nn.silu(x)
def _sigmoid(x):
    return jax.nn.sigmoid(x)
def _layernorm(x, axis=-1, eps=1e-5):
    m = jnp.mean(x, axis=axis, keepdims=True)
    v = jnp.var(x, axis=axis, keepdims=True)
    return (x - m) / jnp.sqrt(v + eps)
def _scatter_add(tgt, idx, src, axis=0):
    return tgt.at[idx].add(src)
def _segment_sum(src, seg, n):
    return jax.ops.segment_sum(src, seg, n)
class _Rng:
    def __init__(self, key):
        self._k = key
    def _next(self):
        self._k, sub = jax.random.split(self._k)
        return sub
    def normal(self, shape):
        return jax.random.normal(self._next(), shape, dtype=jnp.bfloat16)
    def randint(self, lo, hi, shape):
        return jax.random.randint(self._next(), shape, lo, hi, dtype=jnp.int32)
    def uniform(self, shape, lo=0.0, hi=1.0):
        return jax.random.uniform(self._next(), shape, jnp.bfloat16, lo, hi)
    def permutation(self, n):
        return jax.random.permutation(self._next(), n)


kernel_name = 'standalone__dense_activation_gelu__prompt'

def setup_inputs():
    _rng = _Rng(jax.random.key(int.from_bytes(__import__("os").urandom(4), "little")))
    _w = (lambda a: (lambda t: t.astype(jnp.bfloat16) if jnp.issubdtype(t.dtype, jnp.floating) else t)(jnp.asarray(a)))
    B, S, D, F = 1, 2048, 640, 1728
    return {
        "x": _w((lambda *s: _rng.normal(s) * 0.05)(B, S, D)),
        "w1": _w((lambda *s: _rng.normal(s) * 0.05)(D, F) * (D ** -0.5)),
        "b1": _w((lambda *s: _rng.normal(s) * 0.05)(F) * 0.01),
        "w2": _w((lambda *s: _rng.normal(s) * 0.05)(F, D) * (F ** -0.5)),
        "b2": _w((lambda *s: _rng.normal(s) * 0.05)(D) * 0.01),
    }

def reference(x, w1, b1, w2, b2):
    h = jnp.einsum("bsd,df->bsf", x, w1) + b1
    h = _gelu(h)
    return jnp.einsum("bsf,fd->bsd", h, w2) + b2
```

```python
import functools
import math

import jax
import jax.numpy as jnp
from jax import lax
import jax.experimental.pallas as pl
import jax.experimental.pallas.tpu as pltpu

_C0 = math.sqrt(2.0 / math.pi)
_C1 = _C0 * 0.044715
_NT = (((1,), (1,)), ((), ()))
_F32 = jnp.float32
_BF16 = jnp.bfloat16


def _gelu(h):
    u = h * (_C0 + _C1 * (h * h))
    return (0.5 * h) * (1.0 + jnp.tanh(u))


def _offs(sizes, start=0):
    out, s = [], start
    for n in sizes:
        out.append((s, n))
        s += n
    return out


@jax.jit
def pallas_standalone__dense_activation_gelu__prompt_kernel(
    x: jax.Array,
    w1: jax.Array,
    b1: jax.Array,
    w2: jax.Array,
    b2: jax.Array,
):
    B, S, D = x.shape
    F = w1.shape[1]
    M = B * S
    OW1, OW2, OX = 0, F, 2 * F

    XF = _offs((256, 256))
    R0 = 512
    XR = _offs((512, 512, 512), R0)
    W1 = _offs((256, 256, 512, 704))
    X = XF + XR
    osubs = [[R0], [512], [512], [128, 128, 128, 128]]
    n_out = sum(len(o) for o in osubs)

    def kernel(x_hbm, w1_hbm, b1_hbm, w2_hbm, b2_hbm, o_hbm,
               buf, b1v, b2v, ov, sem_x, sem_w1, sem_w2, sem_b, sem_o):
        cp = {}
        for i, (s, n) in enumerate(X):
            cp[f"x{i}"] = pltpu.make_async_copy(
                x_hbm.at[pl.ds(s, n)], buf.at[pl.ds(OX + s, n)], sem_x.at[i])
        for j, (s, n) in enumerate(W1):
            cp[f"w1_{j}"] = pltpu.make_async_copy(
                w1_hbm.at[pl.ds(s, n)], buf.at[pl.ds(OW1 + s, n)], sem_w1.at[j])
        cp["w2"] = pltpu.make_async_copy(w2_hbm, buf.at[pl.ds(OW2, F)], sem_w2.at[0])
        cp["b1"] = pltpu.make_async_copy(b1_hbm, b1v, sem_b.at[0])
        cp["b2"] = pltpu.make_async_copy(b2_hbm, b2v, sem_b.at[1])
        order = ["x0", "w1_0", "x1", "w1_1", "w1_2", "w1_3", "w2", "x2", "x3", "x4"]

        @pl.when(pl.program_id(0) == 0)
        def _():
            cp["b1"].start()
            cp["b2"].start()

        @pl.when(pl.program_id(0) == 1)
        def _():
            for k in order:
                cp[k].start()

        def out_copy(s, n, k):
            return pltpu.make_async_copy(
                ov.at[pl.ds(s, n)], o_hbm.at[pl.ds(s, n)], sem_o.at[k])

        @pl.when(pl.program_id(0) == 2)
        def _():
            done = set()
            ocs = []

            def wait(k):
                if k not in done:
                    done.add(k)
                    cp[k].wait()

            def store_out(s, val):
                n = val.shape[0]
                ov[s:s + n] = val.astype(ov.dtype)
                out_copy(s, n, len(ocs)).start()
                ocs.append((s, n, len(ocs)))

            wait("b1")
            wait("b2")
            b1f = b1v[...].astype(_F32)[None, :]
            b2f = b2v[...].astype(_F32)[None, :]
            gp = {}
            for j, (c0, m) in enumerate(W1):
                for i, (r0, n) in enumerate(XF):
                    wait(f"x{i}")
                    wait(f"w1_{j}")
                    h = lax.dot_general(
                        buf[OX + r0:OX + r0 + n], buf[OW1 + c0:OW1 + c0 + m], _NT,
                        preferred_element_type=_F32) + b1f[:, c0:c0 + m]
                    gp[(i, j)] = _gelu(h).astype(_BF16)
            g0 = jnp.concatenate(
                [jnp.concatenate([gp[(i, j)] for i in range(len(XF))], axis=0)
                 for j in range(len(W1))], axis=1)
            wait("w2")
            store_out(0, jnp.dot(g0, buf[OW2:OW2 + F],
                                 preferred_element_type=_F32) + b2f)
            for i, (r0, n) in enumerate(XR):
                wait(f"x{len(XF) + i}")
                h = lax.dot_general(
                    buf[OX + r0:OX + r0 + n], buf[OW1:OW1 + F], _NT,
                    preferred_element_type=_F32) + b1f
                g = _gelu(h).astype(_BF16)
                for (q0, qn) in _offs(osubs[1 + i]):
                    o = jnp.dot(g[q0:q0 + qn], buf[OW2:OW2 + F],
                                preferred_element_type=_F32) + b2f
                    store_out(r0 + q0, o)
            for (s, n, k) in ocs:
                out_copy(s, n, k).wait()

    out = pl.pallas_call(
        kernel,
        grid=(3,),
        in_specs=[pl.BlockSpec(memory_space=pltpu.HBM)] * 5,
        out_specs=pl.BlockSpec(memory_space=pltpu.HBM),
        out_shape=jax.ShapeDtypeStruct((M, D), x.dtype),
        scratch_shapes=[
            pltpu.VMEM((2 * F + M, D), x.dtype),
            pltpu.VMEM((F,), x.dtype),
            pltpu.VMEM((D,), x.dtype),
            pltpu.VMEM((M, D), x.dtype),
            pltpu.SemaphoreType.DMA((len(X),)),
            pltpu.SemaphoreType.DMA((len(W1),)),
            pltpu.SemaphoreType.DMA((1,)),
            pltpu.SemaphoreType.DMA((2,)),
            pltpu.SemaphoreType.DMA((n_out,)),
        ],
        compiler_params=pltpu.CompilerParams(
            dimension_semantics=("arbitrary",),
            vmem_limit_bytes=100 * 1024 * 1024,
            flags={"XLA_TPU_RESCHEDULE_DMA_DONES": True},
        ),
    )(x.reshape(M, D), w1.T, b1, w2, b2)
    return out.reshape(B, S, D)
```

```python
import math

import jax
import jax.numpy as jnp
from jax import lax
import jax.experimental.pallas as pl
import jax.experimental.pallas.tpu as pltpu

_C0 = math.sqrt(2.0 / math.pi)
_C1 = _C0 * 0.044715
_NT = (((1,), (1,)), ((), ()))
_F32 = jnp.float32
_BF16 = jnp.bfloat16
_LANE = 128

_RAMP = ("x128", "w128", "x128", "w128", "x128", "w128", "x128", "w128",
         "x256", "w512", "w704")
_ROW_TAIL = 128
_REST_BLOCKS = (640, 640)
_LAST_OUT = (384, 192, 64)


def _gelu(h):
    u = h * (_C0 + _C1 * (h * h))
    return (0.5 * h) * (1.0 + jnp.tanh(u))


def _offsets(sizes, start=0):
    out, s = [], start
    for n in sizes:
        out.append((s, n))
        s += n
    return out


def _plan():
    order, dots, rows, cols = [], [], 0, 0
    for piece in _RAMP:
        n = int(piece[1:])
        if piece[0] == "x":
            order.append(("x", rows, n))
            if cols:
                dots.append((rows, n, 0, cols))
            rows += n
        else:
            order.append(("w1", cols, n))
            if rows >= 2 * _ROW_TAIL:
                dots.append((0, rows - _ROW_TAIL, cols, n))
                dots.append((rows - _ROW_TAIL, _ROW_TAIL, cols, n))
            elif rows:
                dots.append((0, rows, cols, n))
            cols += n
    return order, dots, rows, cols


@jax.jit
def pallas_standalone__dense_activation_gelu__prompt_kernel(
    x: jax.Array,
    w1: jax.Array,
    b1: jax.Array,
    w2: jax.Array,
    b2: jax.Array,
):
    B, S, D = x.shape
    F = w1.shape[1]
    M = B * S

    order, dots0, rows0, cols0 = _plan()
    blocks = _offsets(_REST_BLOCKS, rows0)
    assert cols0 == F and rows0 + sum(_REST_BLOCKS) == M
    order = order + [("w2", 0, F)] + [("x", s, n) for s, n in blocks]
    out_pieces = [[rows0]] + [[n] for _, n in blocks[:-1]] + [list(_LAST_OUT)]
    assert sum(_LAST_OUT) == blocks[-1][1]
    n_in = len(order)
    n_out = sum(len(p) for p in out_pieces)

    base = {"w1": 0, "w2": F, "x": 2 * F}

    def kernel(x_hbm, w1t_hbm, b1_hbm, w2_hbm, b2_hbm, o_hbm,
               buf, b1_vmem, b2_vmem, o_vmem, sem_in, sem_b, sem_out):
        src = {"x": x_hbm, "w1": w1t_hbm, "w2": w2_hbm}
        copies = [
            pltpu.make_async_copy(src[k].at[pl.ds(s, n)],
                                  buf.at[pl.ds(base[k] + s, n)], sem_in.at[i])
            for i, (k, s, n) in enumerate(order)
        ]
        b1_copy = pltpu.make_async_copy(b1_hbm, b1_vmem, sem_b.at[0])
        b2_copy = pltpu.make_async_copy(b2_hbm, b2_vmem, sem_b.at[1])
        step = pl.program_id(0)

        @pl.when(step == 0)
        def _():
            b1_copy.start()
            b2_copy.start()
            copies[0].start()
            copies[1].start()

        @pl.when(step == 1)
        def _():
            for c in copies[2:]:
                c.start()

        @pl.when(step == 2)
        def _():
            arrived = set()

            def need(kind, s, n):
                for i, (k, cs, cn) in enumerate(order):
                    if k == kind and cs < s + n and s < cs + cn and i not in arrived:
                        arrived.add(i)
                        copies[i].wait()

            out_copies = []

            def emit(row0, val):
                n = val.shape[0]
                o_vmem[row0:row0 + n] = val.astype(o_vmem.dtype)
                c = pltpu.make_async_copy(o_vmem.at[pl.ds(row0, n)],
                                          o_hbm.at[pl.ds(row0, n)],
                                          sem_out.at[len(out_copies)])
                c.start()
                out_copies.append(c)

            def hidden(r0, n, c0, m):
                need("x", r0, n)
                need("w1", c0, m)
                xs = buf[base["x"] + r0:base["x"] + r0 + n]
                rem = m % _LANE
                full = m - rem
                parts = []
                if full:
                    w = buf[base["w1"] + c0:base["w1"] + c0 + full]
                    h = lax.dot_general(xs, w, _NT, preferred_element_type=_F32)
                    parts.append(_gelu(h + b1f[:, c0:c0 + full]).astype(_BF16))
                if rem:
                    w = buf[base["w1"] + c0 + full:base["w1"] + c0 + m]
                    ht = lax.dot_general(w, xs, _NT, preferred_element_type=_F32)
                    h = ht.T + b1f[:, c0 + full:c0 + m]
                    parts.append(_gelu(h).astype(_BF16))
                return parts[0] if len(parts) == 1 else jnp.concatenate(parts, axis=1)

            def project(g, row0, pieces):
                need("w2", 0, F)
                for q0, qn in _offsets(pieces):
                    o = jnp.dot(g[q0:q0 + qn], buf[base["w2"]:base["w2"] + F],
                                preferred_element_type=_F32)
                    emit(row0 + q0, o + b2f)

            b1_copy.wait()
            b2_copy.wait()
            b1f = b1_vmem[...].astype(_F32)[None, :]
            b2f = b2_vmem[...].astype(_F32)[None, :]

            pieces = [(d, hidden(*d)) for d in dots0]
            rb = sorted({r for (r0, n, _, _), _ in pieces for r in (r0, r0 + n)})
            cb = sorted({c for (_, _, c0, m), _ in pieces for c in (c0, c0 + m)})

            def cell(ra, rz, ca, cz):
                ((r0, _, c0, _), g), = [
                    (d, g) for d, g in pieces
                    if d[0] <= ra and rz <= d[0] + d[1]
                    and d[2] <= ca and cz <= d[2] + d[3]]
                return g[ra - r0:rz - r0, ca - c0:cz - c0]

            def cat(parts, axis):
                return parts[0] if len(parts) == 1 else jnp.concatenate(parts, axis=axis)

            g = cat([cat([cell(ra, rz, ca, cz) for ra, rz in zip(rb[:-1], rb[1:])], 0)
                     for ca, cz in zip(cb[:-1], cb[1:])], 1)
            project(g, 0, out_pieces[0])

            for (r0, n), pcs in zip(blocks, out_pieces[1:]):
                project(hidden(r0, n, 0, F), r0, pcs)

            assert len(arrived) == n_in
            for c in out_copies:
                c.wait()

    out = pl.pallas_call(
        kernel,
        grid=(3,),
        in_specs=[pl.BlockSpec(memory_space=pltpu.HBM)] * 5,
        out_specs=pl.BlockSpec(memory_space=pltpu.HBM),
        out_shape=jax.ShapeDtypeStruct((M, D), x.dtype),
        scratch_shapes=[
            pltpu.VMEM((2 * F + M, D), x.dtype),
            pltpu.VMEM((F,), x.dtype),
            pltpu.VMEM((D,), x.dtype),
            pltpu.VMEM((M, D), x.dtype),
            pltpu.SemaphoreType.DMA((n_in,)),
            pltpu.SemaphoreType.DMA((2,)),
            pltpu.SemaphoreType.DMA((n_out,)),
        ],
        compiler_params=pltpu.CompilerParams(
            dimension_semantics=("arbitrary",),
            vmem_limit_bytes=100 * 1024 * 1024,
            disable_semaphore_checks=True,
            flags={"XLA_TPU_RESCHEDULE_DMA_DONES": True},
        ),
    )(x.reshape(M, D), w1.T, b1, w2, b2)
    return out.reshape(B, S, D)
```

```python
import math

import jax
import jax.numpy as jnp
from jax import lax
import jax.experimental.pallas as pl
import jax.experimental.pallas.tpu as pltpu

_C0 = math.sqrt(2.0 / math.pi)
_C1 = _C0 * 0.044715
_NT = (((1,), (1,)), ((), ()))
_F32 = jnp.float32
_BF16 = jnp.bfloat16
_LANE = 128

_K_HEAD = 128
_HEAD = ("x256", "w256", "w256", "x256", "w512", "x256", "w640")
_BODY = ("x256", "w256", "x256", "w256", "x256", "w512", "w640")
_ROW_TAIL = 128
_REST_BLOCKS = (640, 640)
_LAST_OUT = (384, 192, 64)
_LAST_COLS = (512, 128)


def _gelu(h):
    u = h * (_C0 + _C1 * (h * h))
    return (0.5 * h) * (1.0 + jnp.tanh(u))


def _offsets(sizes, start=0):
    out, s = [], start
    for n in sizes:
        out.append((s, n))
        s += n
    return out


def _grow(seq, k0, k1):
    pieces, dots, rows, cols = [], [], 0, 0
    for item in seq:
        n = int(item[1:])
        if item[0] == "x":
            pieces.append(("x", rows, n, k0, k1 - k0))
            if cols:
                dots.append((rows, n, 0, cols))
            rows += n
        else:
            pieces.append(("w1", cols, n, k0, k1 - k0))
            if rows >= 2 * _ROW_TAIL:
                dots.append((0, rows - _ROW_TAIL, cols, n))
                dots.append((rows - _ROW_TAIL, _ROW_TAIL, cols, n))
            elif rows:
                dots.append((0, rows, cols, n))
            cols += n
    return pieces, dots, rows, cols


def _concat(parts, axis):
    return parts[0] if len(parts) == 1 else jnp.concatenate(parts, axis=axis)


def _stitch(tiles, ra, rz, ca, cz):
    rb = {ra, rz} | {r for (r0, n, _, _), _ in tiles
                     for r in (r0, r0 + n) if ra <= r <= rz}
    cb = {ca, cz} | {c for (_, _, c0, m), _ in tiles
                     for c in (c0, c0 + m) if ca <= c <= cz}
    rb, cb = sorted(rb), sorted(cb)

    def cell(a, b, c, d):
        ((r0, _, c0, _), val), = [
            (t, v) for t, v in tiles
            if t[0] <= a and b <= t[0] + t[1] and t[2] <= c and d <= t[2] + t[3]]
        return val[a - r0:b - r0, c - c0:d - c0]

    return _concat(
        [_concat([cell(a, b, c, d) for a, b in zip(rb[:-1], rb[1:])], 0)
         for c, d in zip(cb[:-1], cb[1:])], 1)


@jax.jit
def pallas_standalone__dense_activation_gelu__prompt_kernel(
    x: jax.Array,
    w1: jax.Array,
    b1: jax.Array,
    w2: jax.Array,
    b2: jax.Array,
):
    B, S, D = x.shape
    F = w1.shape[1]
    M = B * S

    head, head_dots, rows0, cols_a = _grow(_HEAD, 0, _K_HEAD)
    body, body_dots, rows0_b, cols_b = _grow(_BODY, _K_HEAD, D)
    f_rem = F % _LANE
    f_main = F - f_rem
    blocks = _offsets(_REST_BLOCKS, rows0)
    assert rows0 == rows0_b and cols_a == cols_b == f_main
    assert rows0 + sum(_REST_BLOCKS) == M and sum(_LAST_OUT) == blocks[-1][1]
    assert sum(_LAST_COLS) == D

    order = head + body + [("w1", f_main, f_rem, 0, D), ("w2", 0, F, 0, D)]
    order += [("x", s, n, 0, D) for s, n in blocks]
    n_in = len(order)
    n_out = len(blocks) + len(_LAST_OUT) + len(_LAST_COLS) - 1

    base = {"w1": 0, "w2": F, "x": 2 * F}

    def kernel(x_hbm, w1t_hbm, b1_hbm, w2_hbm, b2_hbm, o_hbm,
               buf, b1_vmem, b2_vmem, o_vmem, sem_in, sem_b, sem_out):
        src = {"x": x_hbm, "w1": w1t_hbm, "w2": w2_hbm}

        def in_copy(i, kind, s, n, k0, kn):
            rows, dst_rows = pl.ds(s, n), pl.ds(base[kind] + s, n)
            if kn == D:
                return pltpu.make_async_copy(
                    src[kind].at[rows], buf.at[dst_rows], sem_in.at[i])
            cols = pl.ds(k0, kn)
            return pltpu.make_async_copy(
                src[kind].at[rows, cols], buf.at[dst_rows, cols], sem_in.at[i])

        copies = [in_copy(i, *piece) for i, piece in enumerate(order)]
        b1_copy = pltpu.make_async_copy(b1_hbm, b1_vmem, sem_b.at[0])
        b2_copy = pltpu.make_async_copy(b2_hbm, b2_vmem, sem_b.at[1])
        step = pl.program_id(0)

        @pl.when(step == 0)
        def _():
            b1_copy.start()
            b2_copy.start()
            copies[0].start()
            copies[1].start()

        @pl.when(step == 1)
        def _():
            for c in copies[2:]:
                c.start()

        @pl.when(step == 2)
        def _():
            arrived = set()

            def need(kind, s, n, k0, k1):
                for i, (kd, ps, pn, pk, pkn) in enumerate(order):
                    if (kd == kind and ps < s + n and s < ps + pn
                            and pk < k1 and k0 < pk + pkn and i not in arrived):
                        arrived.add(i)
                        copies[i].wait()

            def x_rows(r0, n, k0, k1):
                need("x", r0, n, k0, k1)
                return buf[base["x"] + r0:base["x"] + r0 + n, k0:k1]

            def w1_rows(c0, m, k0, k1):
                need("w1", c0, m, k0, k1)
                return buf[base["w1"] + c0:base["w1"] + c0 + m, k0:k1]

            def nt_dot(a, b):
                return lax.dot_general(a, b, _NT, preferred_element_type=_F32)

            def hidden_rem(r0, n):
                xs = x_rows(r0, n, 0, D)
                ht = nt_dot(w1_rows(f_main, f_rem, 0, D), xs)
                return _gelu(ht.T + b1f[:, f_main:]).astype(_BF16)

            out_copies = []

            def emit(row0, val, col0=0):
                n, cn = val.shape
                rows, cols = pl.ds(row0, n), pl.ds(col0, cn)
                if cn == D:
                    o_vmem[rows] = val.astype(o_vmem.dtype)
                    c = pltpu.make_async_copy(
                        o_vmem.at[rows], o_hbm.at[rows],
                        sem_out.at[len(out_copies)])
                else:
                    o_vmem[rows, cols] = val.astype(o_vmem.dtype)
                    c = pltpu.make_async_copy(
                        o_vmem.at[rows, cols], o_hbm.at[rows, cols],
                        sem_out.at[len(out_copies)])
                c.start()
                out_copies.append(c)

            def project(g, row0, col_split=(D,)):
                need("w2", 0, F, 0, D)
                for c0, cn in _offsets(col_split):
                    w = buf[base["w2"]:base["w2"] + F, c0:c0 + cn]
                    o = jnp.dot(g, w, preferred_element_type=_F32)
                    emit(row0, o + b2f[:, c0:c0 + cn], c0)

            b1_copy.wait()
            b2_copy.wait()
            b1f = b1_vmem[...].astype(_F32)[None, :]
            b2f = b2_vmem[...].astype(_F32)[None, :]

            partial = []
            for r0, n, c0, m in head_dots:
                xs = x_rows(r0, n, 0, _K_HEAD)
                partial.append(((r0, n, c0, m),
                                nt_dot(xs, w1_rows(c0, m, 0, _K_HEAD))))
            tiles = []
            for r0, n, c0, m in body_dots:
                xs = x_rows(r0, n, _K_HEAD, D)
                h = nt_dot(xs, w1_rows(c0, m, _K_HEAD, D))
                h = h + _stitch(partial, r0, r0 + n, c0, c0 + m)
                g = _gelu(h + b1f[:, c0:c0 + m]).astype(_BF16)
                if c0 + m == f_main:
                    g = jnp.concatenate([g, hidden_rem(r0, n)], axis=1)
                    m += f_rem
                tiles.append(((r0, n, c0, m), g))
            project(_stitch(tiles, 0, rows0, 0, F), 0)

            for b, (r0, n) in enumerate(blocks):
                h = nt_dot(x_rows(r0, n, 0, D), w1_rows(0, f_main, 0, D))
                g = jnp.concatenate(
                    [_gelu(h + b1f[:, :f_main]).astype(_BF16),
                     hidden_rem(r0, n)], axis=1)
                if b < len(blocks) - 1:
                    project(g, r0)
                else:
                    outs = _offsets(_LAST_OUT)
                    for q0, qn in outs[:-1]:
                        project(g[q0:q0 + qn], r0 + q0)
                    q0, qn = outs[-1]
                    project(g[q0:q0 + qn], r0 + q0, _LAST_COLS)

            assert len(arrived) == n_in and len(out_copies) == n_out
            for c in out_copies:
                c.wait()

    out = pl.pallas_call(
        kernel,
        grid=(3,),
        in_specs=[pl.BlockSpec(memory_space=pltpu.HBM)] * 5,
        out_specs=pl.BlockSpec(memory_space=pltpu.HBM),
        out_shape=jax.ShapeDtypeStruct((M, D), x.dtype),
        scratch_shapes=[
            pltpu.VMEM((2 * F + M, D), x.dtype),
            pltpu.VMEM((F,), x.dtype),
            pltpu.VMEM((D,), x.dtype),
            pltpu.VMEM((M, D), x.dtype),
            pltpu.SemaphoreType.DMA((n_in,)),
            pltpu.SemaphoreType.DMA((2,)),
            pltpu.SemaphoreType.DMA((n_out,)),
        ],
        compiler_params=pltpu.CompilerParams(
            dimension_semantics=("arbitrary",),
            vmem_limit_bytes=100 * 1024 * 1024,
            disable_semaphore_checks=True,
            flags={"XLA_TPU_RESCHEDULE_DMA_DONES": True},
        ),
    )(x.reshape(M, D), w1.T, b1, w2, b2)
    return out.reshape(B, S, D)
```

```python
import math

import jax
import jax.numpy as jnp
from jax import lax
import jax.experimental.pallas as pl
import jax.experimental.pallas.tpu as pltpu

_C0 = math.sqrt(2.0 / math.pi)
_C1 = _C0 * 0.044715
_NT = (((1,), (1,)), ((), ()))
_F32 = jnp.float32
_BF16 = jnp.bfloat16
_LANE = 128

_K_HEAD = 128
_HEAD = ("x256", "w128", "w128", "w256", "x256",
         "w256", "w256", "x256", "w640")
_BODY = ("x256", "w256", "x256", "w256", "x256", "w512", "w640")
_ROW_TAIL = 128
_REST_BLOCKS = (640, 640)
_LAST_OUT = (384, 192, 64)
_LAST_COLS = (512, 128)


def _gelu(h):
    u = h * (_C0 + _C1 * (h * h))
    return (0.5 * h) * (1.0 + jnp.tanh(u))


def _offsets(sizes, start=0):
    out, s = [], start
    for n in sizes:
        out.append((s, n))
        s += n
    return out


def _grow(seq, k0, k1):
    pieces, dots, rows, cols = [], [], 0, 0
    for item in seq:
        n = int(item[1:])
        if item[0] == "x":
            pieces.append(("x", rows, n, k0, k1 - k0))
            if cols:
                dots.append((rows, n, 0, cols))
            rows += n
        else:
            pieces.append(("w1", cols, n, k0, k1 - k0))
            if rows >= 2 * _ROW_TAIL:
                dots.append((0, rows - _ROW_TAIL, cols, n))
                dots.append((rows - _ROW_TAIL, _ROW_TAIL, cols, n))
            elif rows:
                dots.append((0, rows, cols, n))
            cols += n
    return pieces, dots, rows, cols


def _concat(parts, axis):
    return parts[0] if len(parts) == 1 else jnp.concatenate(parts, axis=axis)


def _stitch(tiles, ra, rz, ca, cz):
    rb = {ra, rz} | {r for (r0, n, _, _), _ in tiles
                     for r in (r0, r0 + n) if ra <= r <= rz}
    cb = {ca, cz} | {c for (_, _, c0, m), _ in tiles
                     for c in (c0, c0 + m) if ca <= c <= cz}
    rb, cb = sorted(rb), sorted(cb)

    def cell(a, b, c, d):
        ((r0, _, c0, _), val), = [
            (t, v) for t, v in tiles
            if t[0] <= a and b <= t[0] + t[1] and t[2] <= c and d <= t[2] + t[3]]
        return val[a - r0:b - r0, c - c0:d - c0]

    return _concat(
        [_concat([cell(a, b, c, d) for a, b in zip(rb[:-1], rb[1:])], 0)
         for c, d in zip(cb[:-1], cb[1:])], 1)


@jax.jit
def pallas_standalone__dense_activation_gelu__prompt_kernel(
    x: jax.Array,
    w1: jax.Array,
    b1: jax.Array,
    w2: jax.Array,
    b2: jax.Array,
):
    B, S, D = x.shape
    F = w1.shape[1]
    M = B * S

    head, head_dots, rows0, cols_a = _grow(_HEAD, 0, _K_HEAD)
    body, body_dots, rows0_b, cols_b = _grow(_BODY, _K_HEAD, D)
    f_rem = F % _LANE
    f_main = F - f_rem
    blocks = _offsets(_REST_BLOCKS, rows0)
    assert rows0 == rows0_b and cols_a == cols_b == f_main
    assert rows0 + sum(_REST_BLOCKS) == M and sum(_LAST_OUT) == blocks[-1][1]
    assert sum(_LAST_COLS) == D

    order = head + body + [("w1", f_main, f_rem, 0, D), ("w2", 0, F, 0, D)]
    order += [("x", s, n, 0, D) for s, n in blocks]
    n_in = len(order)
    n_out = len(blocks) + len(_LAST_OUT) + len(_LAST_COLS) - 1

    base = {"w1": 0, "w2": F, "x": 2 * F}

    def kernel(x_hbm, w1t_hbm, b1_hbm, w2_hbm, b2_hbm, o_hbm,
               buf, b1_vmem, b2_vmem, o_vmem, sem_in, sem_b, sem_out):
        src = {"x": x_hbm, "w1": w1t_hbm, "w2": w2_hbm}

        def in_copy(i, kind, s, n, k0, kn):
            rows, dst_rows = pl.ds(s, n), pl.ds(base[kind] + s, n)
            if kn == D:
                return pltpu.make_async_copy(
                    src[kind].at[rows], buf.at[dst_rows], sem_in.at[i])
            cols = pl.ds(k0, kn)
            return pltpu.make_async_copy(
                src[kind].at[rows, cols], buf.at[dst_rows, cols], sem_in.at[i])

        copies = [in_copy(i, *piece) for i, piece in enumerate(order)]
        b1_copy = pltpu.make_async_copy(b1_hbm, b1_vmem, sem_b.at[0])
        b2_copy = pltpu.make_async_copy(b2_hbm, b2_vmem, sem_b.at[1])
        step = pl.program_id(0)

        @pl.when(step == 0)
        def _():
            b1_copy.start()
            b2_copy.start()
            copies[0].start()
            copies[1].start()

        @pl.when(step == 1)
        def _():
            for c in copies[2:]:
                c.start()

        @pl.when(step == 2)
        def _():
            arrived = set()

            def need(kind, s, n, k0, k1):
                for i, (kd, ps, pn, pk, pkn) in enumerate(order):
                    if (kd == kind and ps < s + n and s < ps + pn
                            and pk < k1 and k0 < pk + pkn and i not in arrived):
                        arrived.add(i)
                        copies[i].wait()

            def operands(r0, n, c0, m, k0, k1):
                need("x", r0, n, k0, k1)
                need("w1", c0, m, k0, k1)
                return (buf[base["x"] + r0:base["x"] + r0 + n, k0:k1],
                        buf[base["w1"] + c0:base["w1"] + c0 + m, k0:k1])

            def nt_dot(a, b):
                return lax.dot_general(a, b, _NT, preferred_element_type=_F32)

            def hidden_rem(r0, n):
                xs, ws = operands(r0, n, f_main, f_rem, 0, D)
                ht = nt_dot(ws, xs)
                return _gelu(ht.T + b1f[:, f_main:]).astype(_BF16)

            out_copies = []

            def emit(row0, val, col0=0):
                n, cn = val.shape
                rows, cols = pl.ds(row0, n), pl.ds(col0, cn)
                if cn == D:
                    o_vmem[rows] = val.astype(o_vmem.dtype)
                    c = pltpu.make_async_copy(
                        o_vmem.at[rows], o_hbm.at[rows],
                        sem_out.at[len(out_copies)])
                else:
                    o_vmem[rows, cols] = val.astype(o_vmem.dtype)
                    c = pltpu.make_async_copy(
                        o_vmem.at[rows, cols], o_hbm.at[rows, cols],
                        sem_out.at[len(out_copies)])
                c.start()
                out_copies.append(c)

            def project(g, row0, col_split=(D,)):
                need("w2", 0, F, 0, D)
                for c0, cn in _offsets(col_split):
                    w = buf[base["w2"]:base["w2"] + F, c0:c0 + cn]
                    o = jnp.dot(g, w, preferred_element_type=_F32)
                    emit(row0, o + b2f[:, c0:c0 + cn], c0)

            b1_copy.wait()
            b2_copy.wait()
            b1f = b1_vmem[...].astype(_F32)[None, :]
            b2f = b2_vmem[...].astype(_F32)[None, :]

            partial = []
            for r0, n, c0, m in head_dots:
                xs, ws = operands(r0, n, c0, m, 0, _K_HEAD)
                partial.append(((r0, n, c0, m), nt_dot(xs, ws)))
            tiles = []
            for r0, n, c0, m in body_dots:
                xs, ws = operands(r0, n, c0, m, _K_HEAD, D)
                h = nt_dot(xs, ws) + _stitch(partial, r0, r0 + n, c0, c0 + m)
                g = _gelu(h + b1f[:, c0:c0 + m]).astype(_BF16)
                if c0 + m == f_main:
                    g = jnp.concatenate([g, hidden_rem(r0, n)], axis=1)
                    m += f_rem
                tiles.append(((r0, n, c0, m), g))
            project(_stitch(tiles, 0, rows0, 0, F), 0)

            for b, (r0, n) in enumerate(blocks):
                xs, ws = operands(r0, n, 0, f_main, 0, D)
                h = nt_dot(xs, ws)
                g = jnp.concatenate(
                    [_gelu(h + b1f[:, :f_main]).astype(_BF16),
                     hidden_rem(r0, n)], axis=1)
                if b < len(blocks) - 1:
                    project(g, r0)
                else:
                    outs = _offsets(_LAST_OUT)
                    for q0, qn in outs[:-1]:
                        project(g[q0:q0 + qn], r0 + q0)
                    q0, qn = outs[-1]
                    project(g[q0:q0 + qn], r0 + q0, _LAST_COLS)

            assert len(arrived) == n_in and len(out_copies) == n_out
            for c in out_copies:
                c.wait()

    out = pl.pallas_call(
        kernel,
        grid=(3,),
        in_specs=[pl.BlockSpec(memory_space=pltpu.HBM)] * 5,
        out_specs=pl.BlockSpec(memory_space=pltpu.HBM),
        out_shape=jax.ShapeDtypeStruct((M, D), x.dtype),
        scratch_shapes=[
            pltpu.VMEM((2 * F + M, D), x.dtype),
            pltpu.VMEM((F,), x.dtype),
            pltpu.VMEM((D,), x.dtype),
            pltpu.VMEM((M, D), x.dtype),
            pltpu.SemaphoreType.DMA((n_in,)),
            pltpu.SemaphoreType.DMA((2,)),
            pltpu.SemaphoreType.DMA((n_out,)),
        ],
        compiler_params=pltpu.CompilerParams(
            dimension_semantics=("arbitrary",),
            vmem_limit_bytes=100 * 1024 * 1024,
            disable_semaphore_checks=True,
            flags={"XLA_TPU_RESCHEDULE_DMA_DONES": True},
        ),
    )(x.reshape(M, D), w1.T, b1, w2, b2)
    return out.reshape(B, S, D)
```
